```python
import os as _os
_os.environ.setdefault('JAX_PLATFORMS', 'cpu')
import jax
import jax.numpy as jnp

def _softmax(x, axis=-1):
    return jax.nn.softmax(x, axis=axis)

def _gelu(x):
    return jax.nn.gelu(x, approximate=True)

def _silu(x):
    return jax.nn.silu(x)

def _sigmoid(x):
    return jax.nn.sigmoid(x)

def _layernorm(x, axis=-1, eps=1e-05):
    m = jnp.mean(x, axis=axis, keepdims=True)
    v = jnp.var(x, axis=axis, keepdims=True)
    return (x - m) / jnp.sqrt(v + eps)

def _scatter_add(tgt, idx, src, axis=0):
    return tgt.at[idx].add(src)

def _segment_sum(src, seg, n):
    return jax.ops.segment_sum(src, seg, n)

class _Rng:

    def __init__(self, key):
        self._k = key

    def _next(self):
        self._k, sub = jax.random.split(self._k)
        return sub

    def normal(self, shape):
        return jax.random.normal(self._next(), shape, dtype=jnp.bfloat16)

    def randint(self, lo, hi, shape):
        return jax.random.randint(self._next(), shape, lo, hi, dtype=jnp.int32)

    def uniform(self, shape, lo=0.0, hi=1.0):
        return jax.random.uniform(self._next(), shape, jnp.bfloat16, lo, hi)

    def permutation(self, n):
        return jax.random.permutation(self._next(), n)
kernel_name = 'adaLN_cond__mha_block__geglu_ffn__prompt'

def setup_inputs():
    _rng = _Rng(jax.random.key(int.from_bytes(__import__("os").urandom(4), "little")))
    _w = lambda a: (lambda t: t.astype(jnp.bfloat16) if jnp.issubdtype(t.dtype, jnp.floating) else t)(jnp.asarray(a))

    def _A_setup():
        B, S, D, H = (1, 2048, 640, 32)
        return {'x': _w((lambda *s: _rng.normal(s) * 0.05)(B, S, D)), 'wqkv': _w((lambda *s: _rng.normal(s) * 0.05)(D, 3 * D)), 'wo': _w((lambda *s: _rng.normal(s) * 0.05)(D, D))}
    _A_in = _A_setup()

    def _B_setup():
        B, S, D, F = (1, 2048, 640, 1728)
        return {'x': _w((lambda *s: _rng.normal(s) * 0.05)(B, S, D)), 'w_gate': _w((lambda *s: _rng.normal(s) * 0.05)(D, F)), 'w_up': _w((lambda *s: _rng.normal(s) * 0.05)(D, F)), 'w_down': _w((lambda *s: _rng.normal(s) * 0.05)(F, D))}
    _B_in = _B_setup()
    return {'A_x': _A_in['x'], 'A_wqkv': _A_in['wqkv'], 'A_wo': _A_in['wo'], 'B_x': _B_in['x'], 'B_w_gate': _B_in['w_gate'], 'B_w_up': _B_in['w_up'], 'B_w_down': _B_in['w_down'], 'c': _w((lambda *s: _rng.normal(s) * 0.05)(1, 640) * 8.0), 'w_mod': _w((lambda *s: _rng.normal(s) * 0.05)(640, 6 * 640) * 640 ** (-0.5) * 8.0)}

def reference(A_x, A_wqkv, A_wo, B_x, B_w_gate, B_w_up, B_w_down, c, w_mod):

    def _A_ref(x, wqkv, wo):
        B, S, D = x.shape
        H = 32
        Dh = D // H
        qkv = (lambda x, *d: x.transpose(*d))((x @ wqkv).reshape(B, S, 3, H, Dh), 2, 0, 3, 1, 4)
        q, k, v = (qkv[0], qkv[1], qkv[2])
        scores = jnp.einsum('bhqd,bhkd->bhqk', q, k) * Dh ** (-0.5)
        p = _softmax(scores, axis=-1)
        o = jnp.einsum('bhqk,bhkd->bhqd', p, v)
        return (lambda x, *d: x.transpose(*d))(o, 0, 2, 1, 3).reshape(B, S, D) @ wo

    def _B_ref(x, w_gate, w_up, w_down):
        return _gelu(x @ w_gate) * (x @ w_up) @ w_down
    x = A_x
    mod = (_silu(c) @ w_mod).reshape(c.shape[0], 6, 1, -1)
    sa, ca, ga, sb, cb, gb = (mod[:, 0].copy(), mod[:, 1].copy(), mod[:, 2].copy(), mod[:, 3].copy(), mod[:, 4].copy(), mod[:, 5].copy())
    h = _layernorm(x, axis=-1) * (1 + ca) + sa
    x = x + ga * _A_ref(h, A_wqkv, A_wo)
    h = _layernorm(x, axis=-1) * (1 + cb) + sb
    x = x + gb * _B_ref(h, B_w_gate, B_w_up, B_w_down)
    return x
```

```python
import math

import jax
import jax.numpy as jnp
from jax import lax
import jax.experimental.pallas as pl
import jax.experimental.pallas.tpu as pltpu

BF16 = jnp.bfloat16
F32 = jnp.float32
U32 = jnp.uint32

H = 32
QB = 512
KC = 128
RB = 512
EPS = 1e-5


def _layernorm(x):
    mean = jnp.mean(x, axis=-1, keepdims=True)
    xc = x - mean
    var = jnp.mean(xc * xc, axis=-1, keepdims=True)
    return xc * lax.rsqrt(var + EPS)


def _gelu(x):
    c = math.sqrt(2.0 / math.pi)
    return (0.5 * x) * (1.0 + jnp.tanh(x * (c + (c * 0.044715) * (x * x))))


def _dot_nt(a, b):
    return lax.dot_general(a, b, (((1,), (1,)), ((), ())), preferred_element_type=F32)


def _kernel(c_hbm, x_hbm, wqkv_hbm, wo_hbm, wg_hbm, wu_hbm, wd_hbm, wmod_hbm,
            o_hbm,
            c_v, x_v, wqkv_v, wo_v, wg_v, wu_v, wd_v, wmod_v, mod_s,
            kg_s, qt_s, vp_s, ot_s, sa_s, sb_s, ma_s, mb_s, out_s, sems, osems):
    S, D = x_v.shape
    F = wd_v.shape[0]
    DH = D // H
    FM = (F // 128) * 128
    NQ = S // QB
    NR = S // RB

    cp_mod_a = pltpu.make_async_copy(wmod_hbm.at[:, pl.ds(0, 2 * D)], wmod_v.at[:, pl.ds(0, 2 * D)], sems.at[0])
    cp_x0 = pltpu.make_async_copy(x_hbm.at[pl.ds(0, RB)], x_v.at[pl.ds(0, RB)], sems.at[1])
    cp_wqkv = pltpu.make_async_copy(wqkv_hbm, wqkv_v, sems.at[2])
    cp_x1 = pltpu.make_async_copy(x_hbm.at[pl.ds(RB, S - RB)], x_v.at[pl.ds(RB, S - RB)], sems.at[3])
    cp_mod_b = pltpu.make_async_copy(wmod_hbm.at[:, pl.ds(2 * D, 4 * D)], wmod_v.at[:, pl.ds(2 * D, 4 * D)], sems.at[4])
    cp_wo = pltpu.make_async_copy(wo_hbm, wo_v, sems.at[5])
    cp_wg = pltpu.make_async_copy(wg_hbm, wg_v, sems.at[6])
    cp_wu = pltpu.make_async_copy(wu_hbm, wu_v, sems.at[7])
    cp_wd = pltpu.make_async_copy(wd_hbm, wd_v, sems.at[8])

    cp_c = pltpu.make_async_copy(c_hbm, c_v, sems.at[9])
    cp_c.start()
    cp_mod_a.start()
    cp_x0.start()
    cp_wqkv.start()

    cp_c.wait()
    cv = c_v[...].astype(F32)
    sc = jnp.broadcast_to(cv * (1.0 / (1.0 + jnp.exp(-cv))), (16, D)).astype(BF16)
    cp_mod_a.wait()
    cp_x1.start()
    mod_s[:, pl.ds(0, 2 * D)] = jnp.dot(sc, wmod_v[:, pl.ds(0, 2 * D)], preferred_element_type=F32)[:8]
    cp_x0.wait()
    cp_wqkv.wait()
    for cp in (cp_mod_b, cp_wo, cp_wg, cp_wu, cp_wd):
        cp.start()

    qscale = (DH ** -0.5) * math.log2(math.e)

    def qkv_block(i):
        r0 = i * RB
        rows = pl.ds(r0, RB)
        x = x_v[rows, :].astype(F32)
        h = _layernorm(x) * (1.0 + mod_s[0:1, pl.ds(D, D)]) + mod_s[0:1, pl.ds(0, D)]
        h = h.astype(BF16)
        q = jnp.dot(h, wqkv_v[:, pl.ds(0, D)], preferred_element_type=F32) * qscale
        qt_s[:, rows] = pltpu.bitcast(q.T.astype(BF16), U32)
        k = jnp.dot(h, wqkv_v[:, pl.ds(D, D)], preferred_element_type=F32)
        lane = lax.broadcasted_iota(jnp.int32, (RB, 128), 1)
        for g in range(D // 128):
            kg = k[:, g * 128:(g + 1) * 128]
            kg_s[2 * g, rows, :] = kg.astype(BF16)
            if g + 1 < D // 128:
                kn = k[:, (g + 1) * 128:(g + 2) * 128]
                kg_s[2 * g + 1, rows, :] = jnp.where(lane < 64, kn, kg).astype(BF16)
        v = jnp.dot(h, wqkv_v[:, pl.ds(2 * D, D)], preferred_element_type=F32)
        vt = v.astype(BF16).astype(F32).T
        sub = lax.broadcasted_iota(jnp.int32, (8, RB), 0)
        for p in range(H // 2):
            b = 2 * DH * p
            mid = vt[b + 16:b + 24]
            vp_s[2 * p, 0:16, rows] = vt[b:b + 16]
            vp_s[2 * p, 16:24, rows] = jnp.where(sub < 4, mid, 1.0)
            vp_s[2 * p + 1, 0:8, rows] = jnp.where(sub < 4, 1.0, mid)
            vp_s[2 * p + 1, 8:24, rows] = vt[b + 24:b + 40]

    qkv_block(0)
    cp_x1.wait()

    @pl.loop(1, NR)
    def _(i):
        qkv_block_dyn = pl.multiple_of(i * RB, RB) // RB
        del qkv_block_dyn
        qkv_block(i)

    def group_of(h):
        lo = h * DH
        g = lo // 128
        straddle = ((lo + DH - 1) // 128) - g
        return g, straddle

    def q_weights(h, j):
        g, st = group_of(h)
        cols = pl.ds(pl.multiple_of(j * QB, QB), QB)
        r_lo = pl.multiple_of((g + st) * 64, 32)
        r_hi = pl.multiple_of(g * 64 + 32, 32)
        lo = qt_s[pl.ds(r_lo, 32), cols]
        hi = qt_s[pl.ds(r_hi, 32), cols]
        row = lax.broadcasted_iota(jnp.int32, (32, QB), 0)
        a, b = h * (DH // 2), (h + 1) * (DH // 2)
        lo = jnp.where((row + r_lo >= a) & (row + r_lo < b), lo, jnp.uint32(0))
        hi = jnp.where((row + r_hi >= a) & (row + r_hi < b), hi, jnp.uint32(0))
        return pltpu.bitcast(jnp.concatenate([lo, hi], axis=0), BF16), 2 * g + st

    def stage(nxt, cur, s_in, m_in, s_out, m_out):
        if nxt is not None:
            q, grp = q_weights(*nxt)
        if cur is not None:
            m = m_in[...]
        mx = None
        acc = None
        for c in range(S // KC):
            sl = pl.ds(c * KC, KC)
            if nxt is not None:
                s = jnp.dot(kg_s[grp, sl, :], q, preferred_element_type=F32)
                s_out[sl, :] = s
                cm = jnp.max(s.reshape(KC // 8, 8, QB), axis=0)
                mx = cm if mx is None else jnp.maximum(mx, cm)
            if cur is not None:
                p = jnp.exp2(s_in[sl, :].reshape(KC // 8, 8, QB) - m[None])
                p = p.reshape(KC, QB).astype(BF16)
                o = jnp.dot(vp_s[cur, :, sl], p, preferred_element_type=F32)
                acc = o if acc is None else acc + o
        if nxt is not None:
            m_out[...] = jnp.broadcast_to(jnp.max(mx, axis=0, keepdims=True), (8, QB))
        return acc

    def pair_unit(u, last):
        p, j = u // NQ, u % NQ
        e = stage((2 * p + 1, j), 2 * p, sa_s, ma_s, sb_s, mb_s)
        nxt = None if last else (2 * ((u + 1) // NQ), (u + 1) % NQ)
        o = stage(nxt, 2 * p + 1, sb_s, mb_s, sa_s, ma_s)
        ie = 1.0 / e[DH:DH + 1]
        io = 1.0 / o[0:1]
        e = e * ie
        o = o * io
        sub = lax.broadcasted_iota(jnp.int32, (8, QB), 0)
        res = jnp.concatenate([e[0:16], jnp.where(sub < 4, e[16:24], o[0:8]), o[8:24]], axis=0)
        ot_s[pl.ds(pl.multiple_of(p * 2 * DH, 8), 2 * DH), pl.ds(pl.multiple_of(j * QB, QB), QB)] = res

    stage((0, 0), None, None, None, sa_s, ma_s)
    NU = (H // 2) * NQ

    @pl.loop(0, NU - 1)
    def _(u):
        pair_unit(u, False)

    pair_unit(jnp.int32(NU - 1), True)

    cp_mod_b.wait()
    mod_s[:, pl.ds(2 * D, 4 * D)] = jnp.dot(sc, wmod_v[:, pl.ds(2 * D, 4 * D)], preferred_element_type=F32)[:8]
    cp_wo.wait()
    cp_wg.wait()
    cp_wu.wait()
    cp_wd.wait()

    def out_copy(i):
        rows = pl.ds(pl.multiple_of(i * RB, RB), RB)
        return pltpu.make_async_copy(out_s.at[rows], o_hbm.at[rows], osems.at[i])

    @pl.loop(0, NR)
    def _(i):
        rows = pl.ds(pl.multiple_of(i * RB, RB), RB)
        o = ot_s[:, rows].T.astype(BF16)
        a = jnp.dot(o, wo_v[...], preferred_element_type=F32)
        x1 = x_v[rows, :].astype(F32) + mod_s[0:1, pl.ds(2 * D, D)] * a
        h = _layernorm(x1) * (1.0 + mod_s[0:1, pl.ds(4 * D, D)]) + mod_s[0:1, pl.ds(3 * D, D)]
        h = h.astype(BF16)
        g = _dot_nt(h, wg_v[pl.ds(0, FM), :])
        u = _dot_nt(h, wu_v[pl.ds(0, FM), :])
        act = (_gelu(g) * u).astype(BF16)
        t = _dot_nt(h, jnp.concatenate([wg_v[pl.ds(FM, F - FM), :], wu_v[pl.ds(FM, F - FM), :]], axis=0))
        tl = (_gelu(t) * pltpu.roll(t, 64, 1))[:, :F - FM].astype(BF16)
        y = jnp.dot(act, wd_v[pl.ds(0, FM), :], preferred_element_type=F32)
        y = y + jnp.dot(tl, wd_v[pl.ds(FM, F - FM), :], preferred_element_type=F32)
        out_s[rows, :] = (x1 + mod_s[0:1, pl.ds(5 * D, D)] * y).astype(out_s.dtype)
        out_copy(i).start()

    for i in range(NR):
        out_copy(i).wait()


@jax.jit
def pallas_adaLN_cond__mha_block__geglu_ffn__prompt_kernel(
    A_x, A_wqkv, A_wo, B_x, B_w_gate, B_w_up, B_w_down, c, w_mod,
):
    del B_x
    B, S, D = A_x.shape
    F = B_w_gate.shape[1]
    dt = A_x.dtype
    hbm = pl.BlockSpec(memory_space=pltpu.HBM)
    out = pl.pallas_call(
        _kernel,
        out_shape=jax.ShapeDtypeStruct((S, D), dt),
        in_specs=[hbm] * 8,
        out_specs=hbm,
        scratch_shapes=[
            pltpu.VMEM(c.shape, dt),
            pltpu.VMEM((S, D), dt),
            pltpu.VMEM((D, 3 * D), dt),
            pltpu.VMEM((D, D), dt),
            pltpu.VMEM((F, D), dt),
            pltpu.VMEM((F, D), dt),
            pltpu.VMEM((F, D), dt),
            pltpu.VMEM((D, 6 * D), dt),
            pltpu.VMEM((8, 6 * D), F32),
            pltpu.VMEM((2 * (D // 128) - 1, S, 128), BF16),
            pltpu.VMEM((D // 2, S), U32),
            pltpu.VMEM((H, 24, S), F32),
            pltpu.VMEM((D, S), F32),
            pltpu.VMEM((S, QB), F32),
            pltpu.VMEM((S, QB), F32),
            pltpu.VMEM((8, QB), F32),
            pltpu.VMEM((8, QB), F32),
            pltpu.VMEM((S, D), dt),
            pltpu.SemaphoreType.DMA((10,)),
            pltpu.SemaphoreType.DMA((S // RB,)),
        ],
        compiler_params=pltpu.CompilerParams(vmem_limit_bytes=100 * 2**20),
        name="adaln_block",
    )(c, A_x.reshape(S, D), A_wqkv, A_wo, B_w_gate.T, B_w_up.T, B_w_down, w_mod)
    return out.reshape(B, S, D)
```

```python
import functools
import math

import jax
import jax.numpy as jnp
from jax import lax
import jax.experimental.pallas as pl
import jax.experimental.pallas.tpu as pltpu

BF16 = jnp.bfloat16
F32 = jnp.float32
U32 = jnp.uint32

H = 32
EPS = 1e-5
QB = 512
KC = 128
STEP = 2
RB = 512
OB = 128

GRID = 2.0 ** -8
ROUND = 1.5 * 2.0 ** 23 * GRID
MAX_SCORE = 56.0


def _layernorm(x):
    mean = jnp.mean(x, axis=-1, keepdims=True)
    xc = x - mean
    var = jnp.mean(xc * xc, axis=-1, keepdims=True)
    return xc * lax.rsqrt(var + EPS)


def _gelu(x):
    c = math.sqrt(2.0 / math.pi)
    hx = 0.5 * x
    return hx + hx * jnp.tanh(x * (c + (c * 0.044715) * (x * x)))


def _dot(a, b):
    return jnp.dot(a, b, preferred_element_type=F32)


def _dot_nt(a, b):
    return lax.dot_general(a, b, (((1,), (1,)), ((), ())), preferred_element_type=F32)


def _pack(x):
    return pltpu.bitcast(x.astype(BF16), U32)


def _unpack(x):
    return pltpu.bitcast(x, BF16)


def _transposed(x):
    return x.astype(BF16).T.astype(F32)


def _after(x, dep, never):
    if dep is None:
        return x
    r, c = x.shape
    if (r, c) != (8, 128):
        never = jnp.tile(never.astype(jnp.int32), (r // 8, c // 128)) != 0
        dep = jnp.tile(dep, (r // 8, c // 128))
    return jnp.where(never, dep if dep.dtype == x.dtype else pltpu.bitcast(dep, x.dtype), x)


def _spread(res, n):
    r, c = res.shape
    out = []
    for i in range(n):
        t, g = divmod((i * (r // 8) * (c // 128)) // n, r // 8)
        out.append(res[8 * g:8 * g + 8, 128 * t:128 * t + 128])
    return out


def _spread_over(results, n):
    out = []
    for i, res in enumerate(results):
        k = (n * (i + 1)) // len(results) - (n * i) // len(results)
        out += _spread(res[:, :128], k)
    return out


def _left_operands(a11, a12, a21, a22):
    return [a11 + a22, a21 + a22, a11, a22, a11 + a12, a21 - a11, a12 - a22]


def _right_sums(b11, b12, b21, b22):
    return [b11 + b22, b12 - b22, b21 - b11, b11 + b12, b21 + b22]


def _right_sums_640(top, bot):
    sums = _right_sums(top[:, :256], top[:, 384:], bot[:, :256], bot[:, 384:])
    mid = top[:, 256:384] - bot[:, 256:384]
    sums[1] = jnp.concatenate([mid, sums[1]], axis=1)
    sums[2] = jnp.concatenate([sums[2], -mid], axis=1)
    return sums


def _right_operands_640(sums_ref, top, bot):
    right = [_unpack(sums_ref[m, :, 0:(384 if m in (1, 2) else 256)]) for m in range(5)]
    right.insert(1, top[:, 0:384])
    right.insert(4, bot[:, 256:640])
    return right


def _top_640(m):
    return jnp.concatenate([m[0] + m[3][:, :256] - m[4][:, 128:] + m[6], m[2] + m[4]], axis=1)


def _bottom_640(m):
    return jnp.concatenate([m[1] + m[3], m[0] - m[1][:, :256] + m[2][:, 128:] + m[5]], axis=1)


def _paired_operand(first, second):
    sub = lax.broadcasted_iota(jnp.int32, (8, first.shape[1]), 0)
    const = [jnp.where(sub == 0, c, 0.0) for c in (ROUND, -ROUND)]
    return jnp.concatenate([first] + const + [second], axis=0)


def _unpair(both, grow):
    first = (both + ROUND) - ROUND
    return first, (both - first) * grow


def _kernel(c_hbm, x_hbm, wqkv_hbm, wo_hbm, wg_hbm, wu_hbm, wd_hbm, wmod_hbm, o_hbm,
            x_v, wqkv_v, wo_v, wg_v, wu_v, wd_v, wmod_v, cb_s, mod_s, h_s, x1_s, kt_s, kp_s, kn_s,
            kmax_s, qt_s, qm_s, grow_s, vt_s, ot_s, s_s, p_s, acc_s, chk_s, wo_s, wk_s, qv_s, gu_s,
            dn_s, hl_s, al_s, out_s, c_v, sems, osems):
    S, D = x_v.shape
    F = wd_v.shape[0]
    DH = D // H
    NP = H // 2
    NQ, NR, NC, NT = S // QB, S // RB, S // KC, QB // 128
    HB = RB // 2
    FM = (F // 128) * 128
    NJ = FM // 256
    FH = (NJ + 1) * 128

    def col_copy(src, dst, lo, n, i):
        return pltpu.make_async_copy(src.at[:, pl.ds(lo, n)], dst.at[:, pl.ds(lo, n)], sems.at[i])

    def row_copy(src, dst, lo, n, i):
        return pltpu.make_async_copy(src.at[pl.ds(lo, n)], dst.at[pl.ds(lo, n)], sems.at[i])

    cp_c = pltpu.make_async_copy(c_hbm, c_v.at[0], sems.at[0])
    cp_x0 = row_copy(x_hbm, x_v, 0, RB, 1)
    cp_scale = col_copy(wmod_hbm, wmod_v, D, D, 2)
    cp_wk = col_copy(wqkv_hbm, wqkv_v, D, D, 3)
    cp_shift = col_copy(wmod_hbm, wmod_v, 0, D, 4)
    cp_wq = col_copy(wqkv_hbm, wqkv_v, 0, D, 5)
    cp_wv = col_copy(wqkv_hbm, wqkv_v, 2 * D, D, 6)
    cp_x1 = row_copy(x_hbm, x_v, RB, RB, 7)
    cp_x2 = row_copy(x_hbm, x_v, 2 * RB, S - 2 * RB, 8)
    cp_later = [pltpu.make_async_copy(wg_hbm, wg_v, sems.at[9]), pltpu.make_async_copy(wu_hbm, wu_v, sems.at[10]),
                pltpu.make_async_copy(wd_hbm, wd_v, sems.at[11]), col_copy(wmod_hbm, wmod_v, 2 * D, 4 * D, 12),
                pltpu.make_async_copy(wo_hbm, wo_v, sems.at[13])]
    for cp in [cp_c, cp_x0, cp_scale, cp_wk, cp_shift, cp_wq, cp_wv, cp_x1, cp_x2] + cp_later:
        cp.start()

    def mod(k):
        return mod_s[0:1, pl.ds(k * D, D)]

    def normalize(load, k, buf, r, deps):
        halves = []
        for half, dep in enumerate(deps):
            x = load(half).astype(F32)
            x = jnp.concatenate([_after(x[:, :128], dep, never), x[:, 128:]], axis=1)
            halves.append(_layernorm(x) * (1.0 + mod(k + 1)) + mod(k))
        top, bot = halves
        n = top.shape[0] // 2
        h_s[pl.ds(buf * HB + r // 2, n), :] = _pack(top)
        h_s[pl.ds(buf * HB + HB // 2 + r // 2, n), :] = _pack(bot)
        left = _left_operands(top[:, 0:256], top[:, 256:512], bot[:, 0:256], bot[:, 256:512])
        for m, j in enumerate((0, 1, 4, 5, 6)):
            hl_s.at[buf, m][pl.ds(r // 2, n), :] = _pack(left[j])

    def left_operands(buf):
        top, bot = pl.ds(buf * HB, HB // 2), pl.ds(buf * HB + HB // 2, HB // 2)
        return [_unpack(x) for x in (hl_s[buf, 0], hl_s[buf, 1], h_s[top, 0:256], h_s[bot, 256:512],
                                     hl_s[buf, 2], hl_s[buf, 3], hl_s[buf, 4])]

    q_scale = (DH ** -0.5) * math.log2(math.e)

    def store_k(i, k):
        kt_s[pl.ds(i * HB, HB), :] = _pack(k)
        two = [jnp.concatenate([kt_s[pl.ds(i * HB + r + o, 8), :] for r in range(0, HB, 16)], axis=0)
               for o in (0, 8)]
        lane = lax.broadcasted_iota(jnp.int32, (HB // 2, 128), 1)
        for p in range(NP):
            g, sh = divmod(2 * DH * p, 128)
            moved = []
            for x, to in zip(two, (0, 56)):
                t = x[:, g * 128:(g + 1) * 128]
                if sh + 2 * DH > 128:
                    t = jnp.where(lane < 64, x[:, (g + 1) * 128:(g + 2) * 128], t)
                moved.append(pltpu.roll(t, (to - sh) % 128, 1) if to != sh else t)
            kp_s[p, pl.ds(i * HB // 2, HB // 2), :] = jnp.where(
                lane < 40, moved[0], jnp.where(lane < 56, jnp.uint32(0x3F803F80), moved[1]))

    def store_t(ref, r, x):
        ref[:, :, pl.ds(r, x.shape[0])] = _transposed(x).reshape(NP, 2 * DH, x.shape[0])

    def norm_block(i, deps):
        n = RB // len(deps)
        for z in range(len(deps) // 2):
            normalize(lambda half: x_v[pl.ds(i * RB + half * HB + z * n, n), :], 0, i, z * n, deps[2 * z:2 * z + 2])

    def prep_k(deps):
        n = 256 // len(deps)
        for z, dep in enumerate(deps):
            top, bot = (wqkv_v[pl.ds(r + z * n, n), D:2 * D].astype(F32) for r in (0, 256))
            top = jnp.concatenate([_after(top[:, :384], dep, never), top[:, 384:]], axis=1)
            bot = jnp.concatenate([bot[:, :384], _after(bot[:, 384:], dep, never)], axis=1)
            for m, f in enumerate(_right_sums_640(top, bot)):
                wk_s.at[m][pl.ds(z * n // 2, n // 2), 0:f.shape[1]] = _pack(f)

    def prep_qv(deps):
        n = 256 // len(deps)
        for z, dep in enumerate(deps):
            q1, q2, v1, v2 = (wqkv_v[pl.ds(r + z * n, n), pl.ds(c0, D)].astype(F32)
                              for c0 in (0, 2 * D) for r in (0, 256))
            for m, f in enumerate(_right_sums(_after(q1, dep, never), v1, q2, _after(v2, dep, never))):
                qv_s.at[m][pl.ds(z * n // 2, n // 2), :] = _pack(f)

    def proj_first(c0):
        return _dot(_unpack(h_s[pl.ds(0, HB), :]), wqkv_v[:, pl.ds(c0, D)])

    def proj_k(i):
        right = _right_operands_640(wk_s, wqkv_v.at[0:256, D:2 * D], wqkv_v.at[256:512, D:2 * D])
        m = [_dot(a, b) for a, b in zip(left_operands(i), right)]
        rest = _dot(_unpack(h_s[pl.ds(i * HB, HB), 512:D]), wqkv_v[512:D, D:2 * D])
        store_k(i, jnp.concatenate([_top_640(m) + rest[:HB], _bottom_640(m) + rest[HB:]], axis=0))
        return m

    def proj_qv(i):
        left = left_operands(i)
        top, bot = (_unpack(h_s[pl.ds(i * HB + r, HB // 2), 512:D]) for r in (0, HB // 2))
        right = [_unpack(qv_s[m]) for m in range(5)]
        right.insert(1, wqkv_v[0:256, 0:D])
        right.insert(4, wqkv_v[256:512, 2 * D:3 * D])
        m = [_dot(left[k], right[k]) for k in range(5)]
        rest = _dot(bot, wqkv_v[512:D, 0:D])
        store_t(qt_s, i * RB + HB, (m[1] + m[3] + rest) * q_scale)
        store_t(vt_s, i * RB, m[2] + m[4] + _dot(top, wqkv_v[512:D, 2 * D:3 * D]))
        m5 = _dot(jnp.concatenate([left[5], bot], axis=1),
                  jnp.concatenate([right[5], wqkv_v[512:D, 2 * D:3 * D]], axis=0))
        store_t(vt_s, i * RB + HB, m[0] - m[1] + m[2] + m5)
        m6 = _dot(jnp.concatenate([left[6], top], axis=1), jnp.concatenate([right[6], wqkv_v[512:D, 0:D]], axis=0))
        store_t(qt_s, i * RB, (m[0] + m[3] - m[4] + m6) * q_scale)
        return m + [rest, m5]

    cp_c.wait()
    cv = c_v[0].astype(F32)
    silu_c = jnp.broadcast_to(cv * (1.0 / (1.0 + jnp.exp(-cv))), (16, D)).astype(BF16)

    tmp0, tmp1 = x1_s.at[pl.ds(0, RB)], x1_s.at[pl.ds(RB, RB)]
    cp_x0.wait()
    tmp0[...] = _layernorm(x_v[pl.ds(0, RB), :].astype(F32))
    cp_scale.wait()
    mod_s[:, pl.ds(D, D)] = _dot(silu_c, wmod_v[:, pl.ds(D, D)])
    scaled = tmp0[...] * (1.0 + mod(1))
    tmp0[...] = scaled
    h_s[pl.ds(0, HB), :] = _pack(scaled)
    cp_wk.wait()
    tmp1[...] = proj_first(D)
    cp_shift.wait()
    cp_wq.wait()
    never = lax.broadcasted_iota(jnp.int32, (8, 128), 0) > (
        pltpu.bitcast(h_s[0:8, 0:128] | jnp.uint32(8), jnp.int32) & 15)
    shift = _dot(silu_c, wmod_v[:, pl.ds(0, D)])
    mod_s[:, pl.ds(0, D)] = shift
    store_k(0, tmp1[...] + _dot(shift.astype(BF16), wqkv_v[:, pl.ds(D, D)])[0:1])
    h_s[pl.ds(0, HB), :] = _pack(tmp0[...] + shift[0:1])
    q = proj_first(0)
    tmp1[...] = q
    prep_k(_spread(q, 10)[2:])
    cp_wv.wait()
    cp_x1.wait()
    store_t(qt_s, 0, tmp1[...] * q_scale)
    v = proj_first(2 * D)
    tmp0[...] = v
    norm_block(1, _spread(v, 24)[:16])
    cp_x2.wait()
    store_t(vt_s, 0, tmp0[...])
    prep_qv(_spread_over(proj_k(1)[:4], 16))
    norm_block(2, _spread_over(proj_qv(1), 32))
    norm_block(3, _spread_over(proj_k(2) + proj_qv(2)[:4], 32))
    proj_k(3)
    proj_qv(3)

    NU = 2 * NQ

    def head_rows(pair, e, cols, dep=None, never=None):
        q = _after(qt_s[pair, pl.ds(16 * e, 24), cols], dep, never)
        sub, zero = lax.broadcasted_iota(jnp.int32, (8, QB), 0), jnp.zeros((16, QB), F32)
        if e == 0:
            return jnp.concatenate([q[:16], jnp.where(sub < 4, q[16:], 0.0), zero], axis=0)
        return jnp.concatenate([zero, jnp.where(sub < 4, 0.0, q[:8]), q[8:]], axis=0)

    def values(pair, e, keys):
        v = vt_s[pair, pl.ds(16 * e, 24), keys]
        sub = lax.broadcasted_iota(jnp.int32, (8, v.shape[1]), 0)
        if e == 0:
            return jnp.concatenate([v[:16], jnp.where(sub < 4, v[16:], 1.0)], axis=0)
        return jnp.concatenate([jnp.where(sub < 4, 1.0, v[:8]), v[8:]], axis=0)

    def key_norms(pair, slot, z, dep=None, never=None):
        kt = _unpack(_after(kp_s[pair, pl.ds(64 * z, 64), :], dep, never)).T.astype(F32)
        sub = lax.broadcasted_iota(jnp.int32, (8, 128), 0)
        norms = []
        for r0 in (0, 56):
            sq = [kt[r:r + 8] * kt[r:r + 8] for r in range(r0, r0 + 2 * DH, 8)]
            norms.append([jnp.broadcast_to(jnp.sum(x, axis=0, keepdims=True), (8, 128)) for x in (
                sq[0] + sq[1] + jnp.where(sub < 4, sq[2], 0.0), sq[3] + sq[4] + jnp.where(sub < 4, 0.0, sq[2]))])
        for e in range(2):
            kn_s[slot, e, z] = jnp.maximum(norms[0][e], norms[1][e])

    def largest_key(slot, dep=None, never=None):
        for e in range(2):
            x = _after(jnp.max(kn_s[slot, e], axis=0), dep, never)
            kmax_s[slot, e] = jnp.broadcast_to(jnp.max(x, axis=1, keepdims=True), (8, 128))

    def prepare_unit(pair, slot, u, dep=None, never=None):
        e, j = divmod(u, NQ)
        q = head_rows(pair, e, pl.ds(j * QB, QB), dep, never)
        sq = q[16 * e:16 * e + 24] * q[16 * e:16 * e + 24]
        bound2 = jnp.sum(sq, axis=0, keepdims=True) * jnp.tile(kmax_s[slot, e], (1, NT))
        bound2 = jnp.maximum(bound2 * 1.04, 2.0 ** -20)
        r = lax.rsqrt(bound2)
        qm_s.at[slot, u][...] = _pack(_paired_operand(q, q * jnp.tile((0.5 * GRID) * r, (5, 1))))
        grow_s[slot, u] = (2.0 / GRID) * (bound2 * r)
        chk_s[1] = jnp.maximum(chk_s[1], bound2)

    def probs(pair, slot, u, c):
        groups = [(z, w) for z in range(STEP) for w in reversed(range(KC // 32))]
        keys = jnp.concatenate([kp_s[pair, pl.ds((c + z) * KC // 4 + 8 * w, 8), :] for z, w in groups], axis=0)
        both = _dot(_unpack(keys)[:, :96], _unpack(qm_s[slot, u]))
        two = _unpair(both, jnp.tile(grow_s[slot, u], (both.shape[0] // 8, 1)))
        return [jnp.exp2(jnp.concatenate([x[z * KC // 2 + 16 * w:z * KC // 2 + 16 * w + 16]
                                          for w in reversed(range(KC // 32)) for x in two], axis=0))
                for z in range(STEP)]

    def store_out(p, e, cols, acc):
        if e == 0:
            ot_s[p, 0:24, cols] = acc * (1.0 / acc[DH:DH + 1])
        else:
            acc = acc * (1.0 / acc[0:1])
            sub = lax.broadcasted_iota(jnp.int32, (8, QB), 0)
            ot_s[p, 16:24, cols] = jnp.where(sub < 4, ot_s[p, 16:24, cols], acc[0:8])
            ot_s[p, 24:40, cols] = acc[8:24]

    def later_phase_jobs(p, never):
        def gate_up(t, dep):
            z = jnp.minimum(p * (NJ + 1) + t, FM // 16 - 1)
            j, r = z // 16, (z % 16) * 16
            rows = pl.ds(pl.multiple_of(j * 128 + (r // 128) * FH + r % 128, 16), 16)
            g, u = wg_v[rows, 0:512].astype(F32), wu_v[rows, 0:512].astype(F32)
            sums = _right_sums(_after(g[:, :256], dep, never), u[:, :256], g[:, 256:], _after(u[:, 256:], dep, never))
            for m, f in enumerate(sums):
                gu_s.at[m][pl.ds(pl.multiple_of(z * 8, 8), 8), :] = _pack(f)

        def down(t, dep):
            r = jnp.minimum(p * 64 + t * 16, FH - 16)
            top = wd_v[pl.ds(pl.multiple_of(r, 16), 16), :].astype(F32)
            bot = wd_v[pl.ds(pl.multiple_of(jnp.minimum(FH + r, F - 16), 16), 16), :].astype(F32)
            bot = jnp.where(FH + r < F, bot, 0.0)
            top = jnp.concatenate([_after(top[:, :384], dep, never), top[:, 384:]], axis=1)
            bot = jnp.concatenate([bot[:, :384], _after(bot[:, 384:], dep, never)], axis=1)
            for m, f in enumerate(_right_sums_640(top, bot)):
                dn_s.at[m][pl.ds(pl.multiple_of(r // 2, 8), 8), 0:f.shape[1]] = _pack(f)

        def out_weights(dep):
            top, bot = (wo_v[pl.ds(pl.multiple_of(r + p * 16, 16), 16), :].astype(F32) for r in (0, 256))
            for m, f in enumerate(_right_sums_640(_after(top, dep, never), _after(bot, dep, never))):
                wo_s.at[m][pl.ds(pl.multiple_of(p * 8, 8), 8), 0:f.shape[1]] = _pack(f)

        def modulation(k, dep):
            rows = pl.ds(pl.multiple_of(p * (D // NP), 8), D // NP)
            col = _after(cb_s[rows, :], dep, never)
            x = wmod_v[rows, pl.ds(k * D, D)].astype(F32) * jnp.tile(col, (1, D // 128))
            mod_s[pl.ds(8, 8), pl.ds(k * D, D)] += jnp.sum(x.reshape(-1, 8, D), axis=0)

        return ([functools.partial(gate_up, t) for t in range(NJ + 1)] + [functools.partial(down, t) for t in range(4)]
                + [out_weights] + [functools.partial(modulation, k) for k in range(2, 6)])

    cb_s[...] = jnp.broadcast_to(silu_c[0:1].astype(F32), (128, D)).T
    mod_s[pl.ds(8, 8), pl.ds(2 * D, 4 * D)] = jnp.zeros((8, 4 * D), F32)
    chk_s[...] = jnp.zeros(chk_s.shape, F32)
    for z in range(S // 256):
        key_norms(0, 0, z)
    largest_key(0)
    for u in range(NU):
        prepare_unit(0, 0, u)
    for z, pr in enumerate(probs(0, 0, 0, 0)):
        p_s.at[z][...] = _pack(pr)
    for cp in cp_later:
        cp.wait()

    @pl.loop(0, NP // 2)
    def _(i):
        never = lax.broadcasted_iota(jnp.int32, (8, 128), 0) > i + 8
        current = [_unpack(p_s[z]) for z in range(STEP)]
        mass = chk_s[0]
        for slot in range(2):
            p = 2 * i + slot
            p_next = jnp.minimum(p + 1, NP - 1)
            later = later_phase_jobs(p, never)
            jobs = [functools.partial(key_norms, p_next, 1 - slot, z, never=never) for z in range(S // 256)]
            jobs += later[:1] + [functools.partial(largest_key, 1 - slot, never=never)]
            jobs += [functools.partial(prepare_unit, p_next, 1 - slot, u, never=never) for u in range(NU)]
            jobs += later[1:]
            job_at = {(z * 56 // len(jobs)) * STEP: job for z, job in enumerate(jobs)}
            assert len(job_at) == len(jobs)
            for step in range(0, NU * NC, STEP):
                un, cn = divmod(step + STEP, NC)
                following = probs(p, slot, un, cn) if un < NU else probs(p_next, 1 - slot, 0, 0)
                if step in job_at:
                    job_at[step](following[-1][64:72, 0:128])
                for z, pr in enumerate(current):
                    u, c = divmod(step + z, NC)
                    e, j = divmod(u, NQ)
                    o = _dot(values(p, e, pl.ds(c * KC, KC)), pr.astype(BF16))
                    acc = o if c == 0 else acc_s[...] + o
                    if c < NC - 1:
                        acc_s[...] = acc
                    else:
                        mass = mass + jnp.abs(acc[0:8]) + jnp.abs(acc[8:16]) + jnp.abs(acc[16:24])
                        store_out(p, e, pl.ds(j * QB, QB), acc)
                current = following
        for z, pr in enumerate(current):
            p_s.at[z][...] = _pack(pr)
        chk_s[0] = mass

    mod_s[0:1, pl.ds(2 * D, 4 * D)] = jnp.sum(mod_s[pl.ds(8, 8), pl.ds(2 * D, 4 * D)], axis=0, keepdims=True)

    probe = lax.broadcasted_iota(jnp.int32, (2 * DH, 128), 0) % DH == 0
    probe = _paired_operand(jnp.where(probe, 0.1, 0.0), jnp.where(probe, GRID / 16.0, 0.0)).astype(BF16)
    first, second = _unpair(_dot(jnp.ones((16, probe.shape[0]), BF16), probe)[:8], 8.0 / GRID)
    ordered = (jnp.abs(first - 0.2) < GRID) & (second == 1.0)
    in_range = (chk_s[1] <= MAX_SCORE ** 2) & (chk_s[0] <= 2.0 ** 100)

    @pl.when(jnp.max(jnp.where(in_range, 0.0, 1.0)) + jnp.max(jnp.where(ordered, 0.0, 1.0)) > 0.5)
    def _():
        FC = 256

        @pl.loop(0, NP * NQ)
        def _(i):
            p = i // NQ
            cols = pl.ds(pl.multiple_of((i % NQ) * QB, QB), QB)
            for e in range(2):
                q, zero = head_rows(p, e, cols), jnp.zeros((56, QB), F32)
                qs = [jnp.concatenate(x, axis=0).astype(BF16) for x in ([q, zero], [zero, q])]

                def max_pass(c, m):
                    keys = _unpack(kp_s[p, pl.ds(pl.multiple_of(c * (FC // 4), FC // 4), FC // 4), :])[:, :96]
                    two = [_dot(keys, x) for x in qs]
                    s = jnp.concatenate([x[r:r + 16] for r in range(0, FC // 2, 16) for x in two], axis=0)
                    s_s[pl.ds(pl.multiple_of(c * FC, FC), FC), :] = s
                    return jnp.maximum(m, jnp.max(s, axis=0, keepdims=True))

                row_max = lax.fori_loop(0, S // FC, max_pass, jnp.full((1, QB), -jnp.inf, F32))

                def sum_pass(c, acc):
                    r = pl.ds(pl.multiple_of(c * FC, FC), FC)
                    return acc + _dot(values(p, e, r), jnp.exp2(s_s[r, :] - row_max).astype(BF16))

                store_out(p, e, cols, lax.fori_loop(0, S // FC, sum_pass, jnp.zeros((24, QB), F32)))

    def rows_of(i, r, n):
        return pl.ds(pl.multiple_of(i * RB + r, n), n)

    def out_proj(i, z):
        o = jnp.concatenate([ot_s[:, :, rows_of(i, r + z * OB, OB)].reshape(D, OB) for r in (0, HB)], axis=1)
        for m, x in enumerate(_left_operands(o[0:256, :OB], o[256:512, :OB], o[0:256, OB:], o[256:512, OB:])):
            kt_s[pl.ds((8 * z + m) * OB // 2, OB // 2), 0:256] = pltpu.bitcast(x.astype(BF16).T, U32)
        kt_s[pl.ds(z * OB, OB), 256:384] = pltpu.bitcast(o[512:].astype(BF16).T, U32)
        right = _right_operands_640(wo_s, wo_v.at[0:256], wo_v.at[256:512])
        m = [_dot(_unpack(kt_s[pl.ds((8 * z + k) * OB // 2, OB // 2), 0:256]), b) for k, b in enumerate(right)]
        rest = _dot(_unpack(kt_s[pl.ds(z * OB, OB), 256:384]), wo_v[512:D, :])
        for half, a in enumerate((_top_640(m) + rest[:OB], _bottom_640(m) + rest[OB:])):
            rows = rows_of(i, half * HB + z * OB, OB)
            x1_s[rows, :] = x_v[rows, :].astype(F32) + mod(2) * a
        return m

    def norm_residual(i, deps):
        n = HB // len(deps)
        for z, dep in enumerate(deps):
            normalize(lambda half: x1_s[rows_of(i, half * HB + z * n, n), :], 3, 0, z * n, (dep, dep))

    def out_copy(i, half):
        rows = rows_of(i, half * HB, HB)
        return pltpu.make_async_copy(out_s.at[rows], o_hbm.at[rows], osems.at[i, half])

    def ffn_block(i, more):
        for j in range(NJ + 1):
            if more and j == 2:
                out_proj(i + 1, 0)
            tiles = [pl.ds(j * 128 + r, 128) for r in ((0, FH) if j < NJ else (0,))]
            w = 128 * len(tiles)
            left = left_operands(0)
            right = [_unpack(gu_s[m, pl.ds(j * 128, w // 2), :]) for m in range(5)]
            right.insert(1, jnp.concatenate([wg_v[r, 0:256] for r in tiles], axis=0))
            right.insert(4, jnp.concatenate([wu_v[r, 256:512] for r in tiles], axis=0))
            w_rest = jnp.concatenate([ref[r, 512:D] for ref in (wg_v, wu_v) for r in tiles], axis=0)
            m = [_dot_nt(a, b) for a, b in zip(left[:5], right)]
            rest = _dot_nt(_unpack(h_s[pl.ds(HB // 2, HB // 2), 512:D]), w_rest)
            bot = _gelu(m[1] + m[3] + rest[:, :w]) * (m[0] - m[1] + m[2] + rest[:, w:] + _dot_nt(left[5], right[5]))
            rest = _dot_nt(_unpack(h_s[pl.ds(0, HB // 2), 512:D]), w_rest)
            top = _gelu(m[0] + m[3] - m[4] + rest[:, :w] + _dot_nt(left[6], right[6])) * (m[2] + m[4] + rest[:, w:])
            if j == NJ:
                r = pl.ds(FM, F - FM)
                t = _dot_nt(_unpack(h_s[pl.ds(0, HB), :]), jnp.concatenate([wg_v[r, :], wu_v[r, :]], axis=0))
                lane = lax.broadcasted_iota(jnp.int32, (RB, 128), 1)
                t = jnp.where(lane < F - FM, _gelu(t) * pltpu.roll(t, F - FM, 1), 0.0)
                top, bot = jnp.concatenate([top, t[:HB]], axis=1), jnp.concatenate([bot, t[HB:]], axis=1)
            for k, f in enumerate(_left_operands(top[:, :128], top[:, 128:], bot[:, :128], bot[:, 128:])):
                al_s.at[k][:, pl.ds(j * 128, 128)] = _pack(f)

        def emit(half, y):
            rows = rows_of(i, half * HB, HB)
            out_s[rows, :] = (x1_s[rows, :] + mod(5) * y).astype(out_s.dtype)

        right = _right_operands_640(dn_s, wd_v.at[0:FH], wd_v.at[FH:F])
        if more:
            out_proj(i + 1, 1)
        m = [_dot(_unpack(al_s[k, :, 0:b.shape[0]]), b) for k, b in enumerate(right[:6])]
        if more:
            norm_residual(i + 1, [x for y in m[:4] for x in _spread(y, 4)])
        emit(1, _bottom_640(m))
        if not more:
            out_copy(i, 1).start()
        m.append(_dot(_unpack(al_s[6]), right[6]))
        emit(0, _top_640(m))
        if more:
            out_copy(i, 1).start()
        out_copy(i, 0).start()

    out_proj(0, 0)
    m = out_proj(0, 1)
    norm_residual(0, [m[z * 6 // 8][0:8, 0:128] for z in range(8)] + [None] * 8)
    pl.loop(0, NR - 1)(lambda i: ffn_block(i, True))
    ffn_block(NR - 1, False)
    for i in range(NR):
        out_copy(i, 1).wait()
        out_copy(i, 0).wait()


@jax.jit
def pallas_adaLN_cond__mha_block__geglu_ffn__prompt_kernel(
    A_x: jax.Array,
    A_wqkv: jax.Array,
    A_wo: jax.Array,
    B_x: jax.Array,
    B_w_gate: jax.Array,
    B_w_up: jax.Array,
    B_w_down: jax.Array,
    c: jax.Array,
    w_mod: jax.Array,
):
    del B_x
    B, S, D = A_x.shape
    F = B_w_gate.shape[1]
    assert (B, S, D, F) == (1, 4 * RB, 640, 1728)
    DH = D // H
    dt = A_x.dtype
    fh = (F // 256 + 1) * 128
    hbm = pl.BlockSpec(memory_space=pltpu.HBM)
    scratch = [
        pltpu.VMEM((S, D), dt),
        pltpu.VMEM((D, 3 * D), dt),
        pltpu.VMEM((D, D), dt),
        pltpu.VMEM((F, D), dt),
        pltpu.VMEM((F, D), dt),
        pltpu.VMEM((F, D), dt),
        pltpu.VMEM((D, 6 * D), dt),
        pltpu.VMEM((D, 128), F32),
        pltpu.VMEM((16, 6 * D), F32),
        pltpu.VMEM((S // 2, D), U32),
        pltpu.VMEM((S, D), F32),
        pltpu.VMEM((S // 2, D), U32),
        pltpu.VMEM((H // 2, S // 4, 128), U32),
        pltpu.VMEM((2, 2, S // 256, 8, 128), F32),
        pltpu.VMEM((2, 2, 8, 128), F32),
        pltpu.VMEM((H // 2, 2 * DH, S), F32),
        pltpu.VMEM((2, 2 * S // QB, 48, QB), U32),
        pltpu.VMEM((2, 2 * S // QB, 8, QB), F32),
        pltpu.VMEM((H // 2, 2 * DH, S), F32),
        pltpu.VMEM((H // 2, 2 * DH, S), F32),
        pltpu.VMEM((S, QB), F32),
        pltpu.VMEM((STEP, KC // 2, QB), U32),
        pltpu.VMEM((24, QB), F32),
        pltpu.VMEM((2, 8, QB), F32),
        pltpu.VMEM((5, 128, 384), U32),
        pltpu.VMEM((5, 128, 384), U32),
        pltpu.VMEM((5, 128, D), U32),
        pltpu.VMEM((5, F // 128 * 64, 256), U32),
        pltpu.VMEM((5, fh // 2, 384), U32),
        pltpu.VMEM((S // RB, 5, RB // 4, 256), U32),
        pltpu.VMEM((7, RB // 4, fh), U32),
        pltpu.VMEM((S, D), dt),
        pltpu.VMEM((32,) + c.shape, dt),
        pltpu.SemaphoreType.DMA((14,)),
        pltpu.SemaphoreType.DMA((S // RB, 2)),
    ]
    out = pl.pallas_call(
        _kernel,
        out_shape=jax.ShapeDtypeStruct((S, D), dt),
        in_specs=[hbm] * 8,
        out_specs=hbm,
        scratch_shapes=scratch,
        compiler_params=pltpu.CompilerParams(vmem_limit_bytes=110 * 2**20),
        name="adaln_block",
    )(c, A_x.reshape(S, D), A_wqkv, A_wo, B_w_gate.T, B_w_up.T, B_w_down, w_mod)
    return out.reshape(B, S, D)
```
